```python
import os as _os
_os.environ.setdefault("JAX_PLATFORMS", "cpu")
import jax
import jax.numpy as jnp

def _softmax(x, axis=-1):
    return jax.nn.softmax(x, axis=axis)
def _gelu(x):
    return jax.nn.gelu(x, approximate=True)
def _silu(x):
    return jax.nn.silu(x)
def _sigmoid(x):
    return jax.nn.sigmoid(x)
def _layernorm(x, axis=-1, eps=1e-5):
    m = jnp.mean(x, axis=axis, keepdims=True)
    v = jnp.var(x, axis=axis, keepdims=True)
    return (x - m) / jnp.sqrt(v + eps)
def _scatter_add(tgt, idx, src, axis=0):
    return tgt.at[idx].add(src)
def _segment_sum(src, seg, n):
    return jax.ops.segment_sum(src, seg, n)
class _Rng:
    def __init__(self, key):
        self._k = key
    def _next(self):
        self._k, sub = jax.random.split(self._k)
        return sub
    def normal(self, shape):
        return jax.random.normal(self._next(), shape, dtype=jnp.bfloat16)
    def randint(self, lo, hi, shape):
        return jax.random.randint(self._next(), shape, lo, hi, dtype=jnp.int32)
    def uniform(self, shape, lo=0.0, hi=1.0):
        return jax.random.uniform(self._next(), shape, jnp.bfloat16, lo, hi)
    def permutation(self, n):
        return jax.random.permutation(self._next(), n)


kernel_name = 'gated_mix__grouped_kv_mqa__ssm_conv_s5__prompt'

def setup_inputs():
    _rng = _Rng(jax.random.key(int.from_bytes(__import__("os").urandom(4), "little")))
    _w = (lambda a: (lambda t: t.astype(jnp.bfloat16) if jnp.issubdtype(t.dtype, jnp.floating) else t)(jnp.asarray(a)))
    def _A_setup():
        B, S, D, H = 1, 2048, 512, 32
        Dh = D // H
        return {
            "x": _w((lambda *s: _rng.normal(s) * 0.05)(B, S, D)),
            "wq": _w((lambda *s: _rng.normal(s) * 1.6)(D, H * Dh)),
            "wk": _w((lambda *s: _rng.normal(s) * 1.6)(D, Dh)),
            "wv": _w((lambda *s: _rng.normal(s) * 0.05)(D, Dh)),
            "wo": _w((lambda *s: _rng.normal(s) * 0.05)(H * Dh, D)),
        }
    _A_in = _A_setup()

    def _B_setup():
        B, S, D = 1, 2048, 512
        P = D
        Lambda_re = -0.5 * jnp.exp((lambda *s: _rng.normal(s) * 0.4)(P))
        Lambda_im = (lambda *s: _rng.normal(s) * 0.4)(P) * 1.0
        B_re = (lambda *s: _rng.normal(s) * 0.4)(P, D) * (D ** -0.5)
        B_im = (lambda *s: _rng.normal(s) * 0.4)(P, D) * (D ** -0.5)
        C_re = (lambda *s: _rng.normal(s) * 0.4)(D, P) * (P ** -0.5)
        C_im = (lambda *s: _rng.normal(s) * 0.4)(D, P) * (P ** -0.5)
        log_dt = (lambda *s: _rng.normal(s) * 0.4)(P) * 0.3 - 2.0
        Dskip = (lambda *s: _rng.normal(s) * 0.4)(D)
        return {
            "x": _w((lambda *s: _rng.normal(s) * 0.05)(B, S, D)),
            "Lambda_re": _w(Lambda_re),
            "Lambda_im": _w(Lambda_im),
            "B_re": _w(B_re),
            "B_im": _w(B_im),
            "C_re": _w(C_re),
            "C_im": _w(C_im),
            "log_dt": _w(log_dt),
            "Dskip": _w(Dskip),
        }
    _B_in = _B_setup()

    return {
        "A_x": _A_in["x"],
        "A_wq": _A_in["wq"],
        "A_wk": _A_in["wk"],
        "A_wv": _A_in["wv"],
        "A_wo": _A_in["wo"],
        "B_x": _B_in["x"],
        "B_Lambda_re": _B_in["Lambda_re"],
        "B_Lambda_im": _B_in["Lambda_im"],
        "B_B_re": _B_in["B_re"],
        "B_B_im": _B_in["B_im"],
        "B_C_re": _B_in["C_re"],
        "B_C_im": _B_in["C_im"],
        "B_log_dt": _B_in["log_dt"],
        "B_Dskip": _B_in["Dskip"],
        "gate_w": _w((lambda *s: _rng.normal(s) * 0.05)(512) * 16.0),
    }

def reference(A_x, A_wq, A_wk, A_wv, A_wo, B_x, B_Lambda_re, B_Lambda_im, B_B_re, B_B_im, B_C_re, B_C_im, B_log_dt, B_Dskip, gate_w):
    def _A_ref(x, wq, wk, wv, wo):
        B, S, D = x.shape
        H = 32
        Dh = D // H
        q = (lambda x, *d: x.transpose(*d))((x @ wq).reshape(B, S, H, Dh), 0, 2, 1, 3)
        k = x @ wk
        v = x @ wv
        scores = jnp.einsum("bhqd,bkd->bhqk", q, k) * (Dh ** -0.5)
        p = _softmax(scores, axis=-1)
        o = jnp.einsum("bhqk,bkd->bhqd", p, v)
        return (lambda x, *d: x.transpose(*d))(o, 0, 2, 1, 3).reshape(B, S, H * Dh) @ wo

    def _B_ref(x, Lambda_re, Lambda_im, B_re, B_im, C_re, C_im, log_dt, Dskip):
        Bsz, L, H = x.shape
        Lam = Lambda_re + 1j * Lambda_im
        Bmat = B_re + 1j * B_im
        Cmat = C_re + 1j * C_im
        dt = jnp.exp(log_dt)
        Lam_bar = jnp.exp(dt * Lam)
        B_bar = ((Lam_bar - 1.0) / Lam)[:, None] * Bmat
        Bu = jnp.einsum("bld,pd->blp", x + 0j, B_bar)
        h = jnp.zeros_like(Bu[:, 0, :])
        hs = []
        for t in range(L):
            h = Lam_bar[None, :] * h + Bu[:, t, :]
            hs.append(h)
        hseq = jnp.stack(hs, 1)
        y = 2.0 * jnp.einsum("blp,dp->bld", hseq, Cmat).real + x * Dskip[None, None, :]
        return y

    x = A_x
    g = _sigmoid((x * gate_w).sum(-1, keepdims=True))
    a = _A_ref(x, A_wq, A_wk, A_wv, A_wo)
    b = _B_ref(x, B_Lambda_re, B_Lambda_im, B_B_re, B_B_im, B_C_re, B_C_im, B_log_dt, B_Dskip)
    return g * a + (1 - g) * b
```

```python
import functools
import math

import jax
import jax.numpy as jnp
from jax import lax
import jax.experimental.pallas as pl
import jax.experimental.pallas.tpu as pltpu

S = 2048
D = 512
H = 32
DH = 16
P = 512
BQ = 512
NB = S // BQ
NG = NB * H
BK = 128
NKB = S // BK
KD = 32
UNROLL = 4
LT = P // 128
CH = 32
QSCALE = (DH ** -0.5) * math.log2(math.e)
BOUND_SLACK = 1.0 + 2.0 ** -6
L_SAFE = 2.0 ** -64

f32 = jnp.float32
bf16 = jnp.bfloat16
i32 = jnp.int32

_NT = (((1,), (1,)), ((), ()))


def _cmul(ar, ai, br, bi):
    return ar * br - ai * bi, ar * bi + ai * br


def _pack(v):
    return pltpu.bitcast(v, i32)


def _unpack(v):
    return pltpu.bitcast(v, bf16)


def _kernel(x_ref, wq_ref, wkt_ref, wvt_ref, lre_ref, lim_ref, ldt_ref, dskip_ref, gw_ref,
            wo_hbm, bre_hbm, bim_hbm, cre_hbm, cim_hbm,
            out_ref,
            wo_ref, bre_ref, bim_ref, cre_ref, cim_ref, sem,
            kaug_ref, vt_ref, par_ref, carry_ref, qaug_ref, p0_ref, p1_ref, ot_ref, lmin_ref,
            ure_ref, uim_ref):
    step = pl.program_id(0)
    copies = [pltpu.make_async_copy(src, dst, sem.at[n]) for n, (src, dst) in enumerate(
        ((bre_hbm, bre_ref), (bim_hbm, bim_ref), (wo_hbm, wo_ref), (cre_hbm, cre_ref),
         (cim_hbm, cim_ref)))]

    @pl.when(step == 0)
    def _main():
        for c in copies:
            c.start()

        x = x_ref[...]
        wkv = jnp.concatenate([wkt_ref[...], wvt_ref[...]], axis=0)
        kvt = lax.dot_general(wkv, x, _NT, preferred_element_type=f32)
        kt = kvt[0:DH].astype(bf16).astype(f32)
        vt_ref[...] = _pack(kvt[DH:2 * DH].astype(bf16))
        kn2 = jnp.max(jnp.sum(kt * kt, axis=0, keepdims=True), axis=1, keepdims=True)
        kmax = jnp.sqrt(kn2) * BOUND_SLACK
        rid = lax.broadcasted_iota(i32, (128 - DH, S), 0)
        kaug_t = jnp.concatenate([kt, jnp.where(rid == 0, 1.0, 0.0)], axis=0)
        kaug_ref[...] = _pack(kaug_t.T.astype(bf16))

        def vec(ref):
            return jnp.broadcast_to(ref[...].astype(f32).reshape(1, P), (8, P))

        lre = vec(lre_ref)
        lim = vec(lim_ref)
        dt = jnp.exp(vec(ldt_ref)).astype(bf16).astype(f32)
        mag = jnp.exp(dt * lre)
        a1 = (mag * jnp.cos(dt * lim), mag * jnp.sin(dt * lim))
        den = lre * lre + lim * lim
        nr = a1[0] - 1.0
        coef = (2.0 * (nr * lre + a1[1] * lim) / den, 2.0 * (a1[1] * lre - nr * lim) / den)
        a2 = _cmul(*a1, *a1)
        a3 = _cmul(*a2, *a1)
        a4 = _cmul(*a2, *a2)
        a8 = _cmul(*a4, *a4)
        a16 = _cmul(*a8, *a8)
        sub = lax.broadcasted_iota(i32, (8, P), 0)
        zero = jnp.zeros((8, P), f32)
        masked = [tuple(jnp.where(sub >= sh, v, zero) for v in a) for sh, a in
                  ((1, a4), (2, a8), (4, a16))]
        pw = (jnp.ones((8, P), f32), zero)
        for sh, a in ((1, a4), (2, a8), (4, a16)):
            nxt = _cmul(*pw, *a)
            pw = tuple(jnp.where((sub & sh) != 0, n, o) for n, o in zip(nxt, pw))
        for r, (vr, vi) in enumerate([a1, a2, a3, a4, coef, *masked, pw]):
            par_ref[2 * r] = vr
            par_ref[2 * r + 1] = vi
        carry_ref[...] = jnp.zeros_like(carry_ref)

        copies[0].wait()
        copies[1].wait()

        def proj(b, carry):
            rows = pl.ds(pl.multiple_of(b * BQ, BQ), BQ)
            xb = x_ref[rows, :]
            q = jnp.dot(xb, wq_ref[...], preferred_element_type=f32) * QSCALE
            qt = q.T.astype(bf16)
            qf = qt.astype(f32).reshape(H, DH, BQ)
            mhat = jnp.sqrt(jnp.sum(qf * qf, axis=1, keepdims=True)) * kmax[None]
            rowid = lax.broadcasted_iota(i32, (H, KD - DH, BQ), 1)
            aug = jnp.where(rowid == 0, -mhat, 0.0).astype(bf16)
            heads = pl.ds(pl.multiple_of(b * H, H), H)
            qaug_ref[heads, 0:DH // 2, :] = _pack(qt.reshape(H, DH, BQ))
            qaug_ref[heads, DH // 2:KD // 2, :] = _pack(aug)
            ur = lax.dot_general(xb, bre_ref[...], _NT, preferred_element_type=f32)
            ui = lax.dot_general(xb, bim_ref[...], _NT, preferred_element_type=f32)
            for c in range(LT):
                ure_ref[c, rows, :] = ur[:, c * 128:(c + 1) * 128]
                uim_ref[c, rows, :] = ui[:, c * 128:(c + 1) * 128]
            return carry

        lax.fori_loop(0, NB, proj, 0)

        sub8 = lax.broadcasted_iota(i32, (8, 128), 0)

        def scan_chunk(n):
            off = pl.multiple_of(n * CH, CH)
            for c in range(LT):
                ls = slice(c * 128, (c + 1) * 128)
                tab = lambda r: (par_ref[2 * r, :, ls], par_ref[2 * r + 1, :, ls])
                idx = [pl.ds(off + j, 8, stride=4) for j in range(4)]
                e = []
                for j in range(4):
                    u = (ure_ref[c, idx[j], :], uim_ref[c, idx[j], :])
                    if j:
                        m = _cmul(*tab(0), *e[-1])
                        u = (m[0] + u[0], m[1] + u[1])
                    e.append(u)
                inc = e[3]
                for r, sh in ((5, 1), (6, 2), (7, 4)):
                    m = _cmul(*tab(r), pltpu.roll(inc[0], sh, 0), pltpu.roll(inc[1], sh, 0))
                    inc = (inc[0] + m[0], inc[1] + m[1])
                cm = _cmul(*tab(8), carry_ref[0, :, ls], carry_ref[1, :, ls])
                g = tuple(jnp.where(sub8 == 0, 0.0, pltpu.roll(v, 1, 0)) + w
                          for v, w in zip(inc, cm))
                for j in range(4):
                    m = _cmul(*tab(j), *g)
                    hj = (e[j][0] + m[0], e[j][1] + m[1])
                    if j == 3:
                        carry_ref[0, :, ls] = jnp.broadcast_to(hj[0][7:8], (8, 128))
                        carry_ref[1, :, ls] = jnp.broadcast_to(hj[1][7:8], (8, 128))
                    o = _cmul(*tab(4), *hj)
                    ure_ref[c, idx[j], :] = o[0]
                    uim_ref[c, idx[j], :] = o[1]

        def stage_a(j, qa, p_wr):
            kb = _unpack(kaug_ref[j * (BK // 2):(j + 1) * (BK // 2), :])[:, 0:KD]
            p = jnp.exp2(jnp.dot(kb, qa, preferred_element_type=f32))
            p_wr[j * (BK // 2):(j + 1) * (BK // 2), :] = _pack(p.astype(bf16))
            return jnp.sum(p.reshape(BK // 8, 8, BQ), axis=0)

        def stage_b(j, p_rd):
            vb = _unpack(vt_ref[:, j * BK:(j + 1) * BK])
            pb = _unpack(p_rd[j * (BK // 2):(j + 1) * (BK // 2), :])
            return jnp.dot(vb, pb, preferred_element_type=f32)

        def head(g_a, p_wr, g_b, l_b, p_rd):
            l = acc = None
            if g_a is not None:
                qa = _unpack(qaug_ref[g_a])
            for j in range(NKB):
                if g_a is not None:
                    bl = stage_a(j, qa, p_wr)
                    l = bl if l is None else l + bl
                if g_b is not None:
                    d = stage_b(j, p_rd)
                    acc = d if acc is None else acc + d
            if g_b is not None:
                ot_ref[pl.ds(pl.multiple_of(g_b * DH, DH), DH), :] = acc / l_b
            if g_a is not None:
                l = jnp.sum(l, axis=0, keepdims=True)
                lmin_ref[...] = jnp.minimum(lmin_ref[...], l)
            return l

        bufs = (p0_ref, p1_ref)
        lmin_ref[...] = jnp.full((8, BQ), jnp.inf, f32)
        l_first = head(0, p0_ref, None, None, None)
        n_loop = (NG - 1) // UNROLL
        chunks_per_body = (S // CH) // n_loop

        def body(t, l):
            for u in range(UNROLL):
                g = t * UNROLL + u
                l = head(g + 1, bufs[(u + 1) % 2], g, l, bufs[u % 2])
                if u < chunks_per_body:
                    scan_chunk(t * chunks_per_body + u)
            return l

        l = lax.fori_loop(0, n_loop, body, l_first)
        n_done = n_loop * chunks_per_body
        for g in range(n_loop * UNROLL, NG):
            l = head(g + 1 if g + 1 < NG else None, bufs[(g + 1) % 2], g, l, bufs[g % 2])
            if n_done < S // CH:
                scan_chunk(n_done)
                n_done += 1
        assert n_done == S // CH

        n_bad = jnp.sum(jnp.where(lmin_ref[...] >= L_SAFE, 0.0, 1.0))

        @pl.when(n_bad > 0.0)
        def _true_max_fallback():
            def tile(g, carry):
                qh = _unpack(qaug_ref[g])[0:DH]

                def scores(j):
                    kb = _unpack(kaug_ref[pl.ds(pl.multiple_of(j * (BK // 2), BK // 2), BK // 2), :])
                    return jnp.dot(kb[:, 0:DH], qh, preferred_element_type=f32)

                m = lax.fori_loop(
                    0, NKB, lambda j, m: jnp.maximum(m, jnp.max(scores(j), axis=0, keepdims=True)),
                    jnp.full((1, BQ), -jnp.inf, f32))

                def pv(j, c):
                    p = jnp.exp2(scores(j) - m)
                    vb = _unpack(vt_ref[:, pl.ds(pl.multiple_of(j * BK, BK), BK)])
                    return (c[0] + jnp.dot(vb, p.astype(bf16), preferred_element_type=f32),
                            c[1] + jnp.sum(p, axis=0, keepdims=True))

                acc, l = lax.fori_loop(0, NKB, pv, (jnp.zeros((DH, BQ), f32), jnp.zeros((1, BQ), f32)))
                ot_ref[pl.ds(pl.multiple_of(g * DH, DH), DH), :] = acc / l
                return carry

            lax.fori_loop(0, NG, tile, 0)

        for c in copies[2:]:
            c.wait()

    rows = pl.ds(pl.multiple_of(step * BQ, BQ), BQ)
    o = ot_ref[pl.ds(pl.multiple_of(step * D, D), D), :].T.astype(bf16)
    a = jnp.dot(o, wo_ref[...], preferred_element_type=f32)
    hre = jnp.concatenate([ure_ref[c, rows, :].astype(bf16) for c in range(LT)], axis=1)
    him = jnp.concatenate([uim_ref[c, rows, :].astype(bf16) for c in range(LT)], axis=1)
    y = (lax.dot_general(hre, cre_ref[...], _NT, preferred_element_type=f32)
         - lax.dot_general(him, cim_ref[...], _NT, preferred_element_type=f32))
    xf = x_ref[rows, :].astype(f32)
    b = y + xf * dskip_ref[...].astype(f32).reshape(1, D)
    g = jax.nn.sigmoid(jnp.sum(xf * gw_ref[...].astype(f32).reshape(1, D), axis=1, keepdims=True))
    out_ref[...] = g * a + (1.0 - g) * b


@jax.jit
def pallas_gated_mix__grouped_kv_mqa__ssm_conv_s5__prompt_kernel(
    A_x, A_wq, A_wk, A_wv, A_wo, B_x, B_Lambda_re, B_Lambda_im, B_B_re, B_B_im, B_C_re, B_C_im,
    B_log_dt, B_Dskip, gate_w,
):
    del B_x
    vmem_args = (A_x.reshape(S, D), A_wq, A_wk.T, A_wv.T, B_Lambda_re, B_Lambda_im, B_log_dt,
                 B_Dskip, gate_w)
    hbm_args = (A_wo, B_B_re, B_B_im, B_C_re, B_C_im)
    full = lambda a: pl.BlockSpec(a.shape, lambda i: (0,) * a.ndim)

    out = pl.pallas_call(
        _kernel,
        grid=(NB,),
        in_specs=[full(a) for a in vmem_args] + [pl.BlockSpec(memory_space=pl.ANY)] * len(hbm_args),
        out_specs=pl.BlockSpec((BQ, D), lambda i: (i, 0)),
        out_shape=jax.ShapeDtypeStruct((S, D), f32),
        scratch_shapes=[
            pltpu.VMEM((D, D), bf16), pltpu.VMEM((P, D), bf16), pltpu.VMEM((P, D), bf16),
            pltpu.VMEM((D, P), bf16), pltpu.VMEM((D, P), bf16),
            pltpu.SemaphoreType.DMA((5,)),
            pltpu.VMEM((S // 2, 128), i32),
            pltpu.VMEM((DH // 2, S), i32),
            pltpu.VMEM((18, 8, P), f32),
            pltpu.VMEM((2, 8, P), f32),
            pltpu.VMEM((NG, KD // 2, BQ), i32),
            pltpu.VMEM((S // 2, BQ), i32),
            pltpu.VMEM((S // 2, BQ), i32),
            pltpu.VMEM((NG * DH, BQ), f32),
            pltpu.VMEM((8, BQ), f32),
            pltpu.VMEM((LT, S, 128), f32),
            pltpu.VMEM((LT, S, 128), f32),
        ],
        compiler_params=pltpu.CompilerParams(
            dimension_semantics=("arbitrary",),
            vmem_limit_bytes=100 * 1024 * 1024,
        ),
        name="gated_mix",
    )(*vmem_args, *hbm_args)
    return out.reshape(1, S, D)
```

```python
import math

import jax
import jax.numpy as jnp
import numpy as np
from jax import lax
import jax.experimental.pallas as pl
import jax.experimental.pallas.tpu as pltpu

S = 2048
D = 512
H = 32
DH = 16
P = 512
BQ = 512
NB = S // BQ
NG = NB * H
BK = 128
NKB = S // BK
KD = 32
LT = P // 128
CH = 32
NCH = BQ // CH

QSCALE = (DH ** -0.5) * math.log2(math.e)
BOUND_SLACK = 1.0 + 2.0 ** -6
HEADROOM = 64.0
L_LO = 2.0 ** -80
L_HI = 2.0 ** 80

NVK = 160
MK = S - NVK
GK = 4
UNROLL = 8
LEAD = 3
CHAIN = 8
LAGA = 4
MBLOCKS = [(o, min(BK, MK - o)) for o in range(0, MK, BK)]
UNITS = [(k0, c) for k0 in range(0, NVK, 8 * GK) for c in range(BQ // 128)]
NA = len(MBLOCKS)
OSPLIT = 4
OR = BQ // OSPLIT
KVPOS = 2

SIGN = np.int32(-2 ** 31)
HI16 = np.int32(-2 ** 16)

f32 = jnp.float32
bf16 = jnp.bfloat16
i32 = jnp.int32

_NT = (((1,), (1,)), ((), ()))


def _cmul(ar, ai, br, bi):
    return ar * br - ai * bi, ar * bi + ai * br


def _pack(v):
    return pltpu.bitcast(v, i32)


def _unpack(v):
    return pltpu.bitcast(v, bf16)


def _gate(bits, tok):
    return bits | (pltpu.bitcast(tok, i32) & SIGN)


def _kernel(x_hbm, wq_hbm, wo_hbm, bre_hbm, bim_hbm, cre_hbm, cim_hbm,
            wkt_ref, wvt_ref, lre_ref, lim_ref, ldt_ref, dskip_ref, gw_ref,
            out_hbm,
            x_ref, wq_ref, wo_ref, bre_ref, bim_ref, cre_ref, cim_ref, isem, osem, out_ref,
            kaug_ref, vt_ref, par_ref, qaug_ref, qf_ref, kb_ref, ones_ref, mh_ref,
            p0_ref, p1_ref, pv0_ref, pv1_ref, ot_ref, lmin_ref, lmax_ref,
            ure_ref, uim_ref, vre_ref, vim_ref, hre_ref, him_ref):
    n_sem = [0]

    def copy(src, dst):
        n_sem[0] += 1
        return pltpu.make_async_copy(src, dst, isem.at[n_sem[0] - 1])

    cx = [copy(x_hbm.at[b * BQ:(b + 1) * BQ], x_ref.at[b * BQ:(b + 1) * BQ]) for b in range(NB)]
    cb = [copy(bre_hbm, bre_ref), copy(bim_hbm, bim_ref)]
    cq = copy(wq_hbm, wq_ref)
    co = [copy(cre_hbm, cre_ref), copy(cim_hbm, cim_ref), copy(wo_hbm, wo_ref)]
    for c in (cx[0], *cb, *cx[1:], cq, *co):
        c.start()

    def vec(ref):
        return jnp.broadcast_to(ref[...].astype(f32).reshape(1, P), (8, P))

    lre = vec(lre_ref)
    lim = vec(lim_ref)
    dt = jnp.exp(vec(ldt_ref)).astype(bf16).astype(f32)
    mag = jnp.exp(dt * lre)
    a1 = (mag * jnp.cos(dt * lim), mag * jnp.sin(dt * lim))
    den = lre * lre + lim * lim
    nr = a1[0] - 1.0
    coef = (2.0 * (nr * lre + a1[1] * lim) / den, 2.0 * (a1[1] * lre - nr * lim) / den)
    a2 = _cmul(*a1, *a1)
    a3 = _cmul(*a2, *a1)
    a4 = _cmul(*a2, *a2)
    a8 = _cmul(*a4, *a4)
    a16 = _cmul(*a8, *a8)
    sub = lax.broadcasted_iota(i32, (8, P), 0)
    zero = jnp.zeros((8, P), f32)
    masked = [tuple(jnp.where(sub >= sh, v, zero) for v in a)
              for sh, a in ((1, a4), (2, a8), (4, a16))]
    pw = (jnp.ones((8, P), f32), zero)
    for sh, a in ((1, a4), (2, a8), (4, a16)):
        pw = tuple(jnp.where((sub & sh) != 0, n, o) for n, o in zip(_cmul(*pw, *a), pw))
    for r, (vr, vi) in enumerate([a1, a2, a3, a4, coef, *masked, pw]):
        par_ref[2 * r] = vr
        par_ref[2 * r + 1] = vi

    sub8 = lax.broadcasted_iota(i32, (8, 128), 0)

    def scan_chunk(u_re, u_im, n, off, carry):
        out = []
        for c in range(LT):
            ls = slice(c * 128, (c + 1) * 128)
            tab = lambda r: (par_ref[2 * r, :, ls], par_ref[2 * r + 1, :, ls])
            e = []
            for j in range(4):
                idx = pl.ds(n * CH + j, 8, stride=4)
                u = (u_re[c, idx, :], u_im[c, idx, :])
                if j:
                    m = _cmul(*tab(0), *e[-1])
                    u = (m[0] + u[0], m[1] + u[1])
                e.append(u)
            inc = e[3]
            for r, sh in ((5, 1), (6, 2), (7, 4)):
                m = _cmul(*tab(r), pltpu.roll(inc[0], sh, 0), pltpu.roll(inc[1], sh, 0))
                inc = (inc[0] + m[0], inc[1] + m[1])
            cm = _cmul(*tab(8), *carry[c])
            g = tuple(jnp.where(sub8 == 0, 0.0, pltpu.roll(v, 1, 0)) + w for v, w in zip(inc, cm))
            for j in range(4):
                m = _cmul(*tab(j), *g)
                hj = (e[j][0] + m[0], e[j][1] + m[1])
                if j == 3:
                    out.append(tuple(jnp.broadcast_to(v[7:8], (8, 128)) for v in hj))
                o = _cmul(*tab(4), *hj)
                idx = pl.ds(off + n * CH + j, 8, stride=4)
                hre_ref[c, idx, :] = o[0]
                him_ref[c, idx, :] = o[1]
        return out

    carry = [(jnp.zeros((8, 128), f32), jnp.zeros((8, 128), f32)) for _ in range(LT)]
    ubufs = ((ure_ref, uim_ref), (vre_ref, vim_ref))

    def scan_block(b, lo, hi):
        nonlocal carry
        for n in range(lo, hi):
            carry = scan_chunk(*ubufs[b % 2], n, b * BQ, carry)

    def bu(b, w_ref, dst):
        u = lax.dot_general(x_ref[b * BQ:(b + 1) * BQ, :], w_ref[...], _NT,
                            preferred_element_type=f32)
        for c in range(LT):
            dst[c] = u[:, c * 128:(c + 1) * 128]

    def kv_setup(kvt):
        p1_ref[...] = jnp.zeros_like(p1_ref)
        pv1_ref[...] = jnp.zeros_like(pv1_ref)
        kt = kvt[0:DH].astype(bf16).astype(f32)
        vt_ref[...] = _pack(kvt[DH:2 * DH].astype(bf16))
        kn2 = jnp.max(jnp.sum(kt * kt, axis=0, keepdims=True), axis=1, keepdims=True)
        rid = lax.broadcasted_iota(i32, (128 - DH, S), 0)
        kaug = jnp.concatenate([kt, jnp.where(rid < KD - DH, 1.0, 0.0)], axis=0).T
        kaug_ref[...] = _pack(kaug.astype(bf16))
        for d in range(DH):
            kb_ref[d] = jnp.broadcast_to(kaug[MK:S, d:d + 1], (NVK, 128))
        hid = lax.broadcasted_iota(i32, (H, D), 0)
        jid = lax.broadcasted_iota(i32, (H, D), 1)
        ones_ref[...] = jnp.where(jid // DH == hid, 1.0, 0.0).astype(bf16)
        return jnp.sqrt(kn2) * BOUND_SLACK

    def q_post1(b, q):
        qt = q.T
        qf_ref[b * H:(b + 1) * H] = qt.reshape(H, DH, BQ)
        qaug_ref[b * H:(b + 1) * H, 0:DH // 2, :] = _pack(qt.astype(bf16)).reshape(H, DH // 2, BQ)
        return (qt * qt).astype(bf16)

    def q_post2(b, q2, kmax):
        n2 = jnp.dot(ones_ref[...], q2, preferred_element_type=f32)
        nm = (HEADROOM - jnp.sqrt(n2) * kmax).astype(bf16).astype(f32)
        bits = pltpu.bitcast(nm * (1.0 / (KD - DH)), i32)
        mh_ref[...] = bits | lax.shift_right_logical(bits, 16)
        for h in range(H):
            qaug_ref[b * H + h, DH // 2:KD // 2, :] = jnp.broadcast_to(mh_ref[h:h + 1, :], (8, BQ))

    cx[0].wait()
    cb[0].wait()
    for b in range(NB):
        if 0 < b <= KVPOS:
            cx[b].wait()
        if b == KVPOS:
            for c in cx[b + 1:]:
                c.wait()
            wkv = jnp.concatenate([wkt_ref[...], wvt_ref[...]], axis=0)
            kvt = lax.dot_general(wkv, x_ref[...], _NT, preferred_element_type=f32)
        if b:
            scan_block(b - 1, 0, NCH)
        bu(b, bre_ref, ubufs[b % 2][0])
        if b == 0:
            cb[1].wait()
        if b == KVPOS:
            kmax = kv_setup(kvt)
        bu(b, bim_ref, ubufs[b % 2][1])
    cq.wait()
    q2s = []
    for b in range(NB):
        q = jnp.dot(x_ref[b * BQ:(b + 1) * BQ, :], wq_ref[...], preferred_element_type=f32) * QSCALE
        q2s.append(q_post1(b, q))
        scan_block(NB - 1, b * NCH // NB, (b + 1) * NCH // NB)
        if b:
            q_post2(b - 1, q2s[b - 1], kmax)
    q_post2(NB - 1, q2s[NB - 1], kmax)

    def view(ref, g, sh):
        if isinstance(g, int):
            return ref
        return ref.at[pl.ds(pl.multiple_of(g >> sh, 8), ref.shape[0] - 8), :]

    def stage_a_mxu(off, n, qa, p_wr, tok, lv):
        kbi = kaug_ref[off // 2:(off + n) // 2, :]
        if tok is not None:
            kbi = jnp.concatenate([_gate(kbi[0:8], tok), kbi[8:]], axis=0)
        kb = _unpack(kbi)[:, 0:KD]
        p = jnp.exp2(jnp.dot(kb, qa, preferred_element_type=f32))
        p_wr[off // 2:(off + n) // 2, :] = _pack(p.astype(bf16))
        bl = jnp.sum(p.reshape(n // 8, 8, BQ), axis=0)
        for c in range(4):
            lv[c] = lv[c] + bl[:, c * 128:(c + 1) * 128]
        return bl

    vtoks = []

    def stage_a_vpu(ui, k0, c, g, p_wr, lv, tok):
        z = g >> (10 + ui)
        gq = g + z
        kk0 = pl.multiple_of(k0 + z, 8)
        cs = slice(c * 128, (c + 1) * 128)
        nm = pltpu.bitcast(qaug_ref[gq, DH // 2:KD // 2, cs] & HI16, f32) * float(KD - DH)
        if vtoks:
            tok = jnp.abs(vtoks[-1]) if tok is None else jnp.abs(vtoks[-1]) + tok
        if tok is not None:
            nm = pltpu.bitcast(_gate(pltpu.bitcast(nm, i32), tok), f32)
        accs = [nm] * GK
        for d in range(DH):
            qb = jnp.broadcast_to(qf_ref[gq, d:d + 1, cs], (8, 128))
            for kk in range(GK):
                accs[kk] = accs[kk] + kb_ref[d, pl.ds(kk0 + 8 * kk, 8), :] * qb
            if d == CHAIN - 1:
                vtoks.append(accs[0])
        ps = [jnp.exp2(a) for a in accs]
        for kk in range(0, GK, 2):
            r = k0 // 2 + 4 * kk
            p_wr[r:r + 8, cs] = _pack(jnp.concatenate([ps[kk], ps[kk + 1]], axis=0).astype(bf16))
        t = ps[0]
        for v in ps[1:]:
            t = t + v
        lv[c] = lv[c] + t

    def stage_b(j, p_rd):
        vb = _unpack(vt_ref[:, j * BK:(j + 1) * BK])
        r0, r1 = j * BK, (j + 1) * BK
        parts = []
        if r0 < MK:
            parts.append(p_rd[0][r0 // 2:min(r1, MK) // 2, :])
        if r1 > MK:
            parts.append(p_rd[1][(max(r0, MK) - MK) // 2:(r1 - MK) // 2, :])
        pb = _unpack(parts[0] if len(parts) == 1 else jnp.concatenate(parts, axis=0))
        return jnp.dot(vb, pb, preferred_element_type=f32)

    pbufs = ((p0_ref, pv0_ref), (p1_ref, pv1_ref))

    def steps(g0, n_steps, do_a, l_prev):
        mtoks, atoks = [], []
        vtoks.clear()
        for u in range(n_steps):
            g_a = g0 + u + 1
            wr, rd = pbufs[u % 2], pbufs[(u + 1) % 2]
            p_rd = [view(rd[0], g_a, 22), view(rd[1], g_a, 24)]
            acc = None
            if do_a:
                p_wr = view(wr[0], g_a, 21)
                pv_wr = view(wr[1], g_a, 23)
                qa = _unpack(qaug_ref[g_a])
                lv = [jnp.zeros((8, 128), f32) for _ in range(4)]
            for j in range(NA):
                if do_a:
                    tok = atoks[-LAGA] if len(atoks) >= LAGA else None
                    bl = stage_a_mxu(*MBLOCKS[j], qa, p_wr, tok, lv)
                    mtoks.append(bl[:, 0:128])
                    atoks.append(bl[:, 0:128] + bl[:, 384:512])
                    for ui in range(len(UNITS)):
                        if (ui * NA) // len(UNITS) == j:
                            tok = mtoks[-LEAD] if len(mtoks) >= LEAD else None
                            stage_a_vpu(ui, *UNITS[ui], g_a, pv_wr, lv, tok)
                for jb in range((j * NKB) // NA, ((j + 1) * NKB) // NA):
                    dd = stage_b(jb, p_rd)
                    acc = dd if acc is None else acc + dd
            ot_ref[pl.ds(pl.multiple_of(g_a * DH, DH), DH), :] = acc / l_prev
            if do_a:
                l_prev = jnp.sum(jnp.concatenate(lv, axis=1), axis=0, keepdims=True)
                lmin_ref[...] = jnp.minimum(lmin_ref[...], l_prev)
                lmax_ref[...] = jnp.maximum(lmax_ref[...], l_prev)
        return l_prev

    lmin_ref[...] = jnp.full((8, BQ), jnp.inf, f32)
    lmax_ref[...] = jnp.zeros((8, BQ), f32)
    l = lax.fori_loop(0, NG // UNROLL, lambda t, l: steps(t * UNROLL - 1, UNROLL, True, l),
                      jnp.ones((1, BQ), f32))
    steps(NG - 1, 1, False, l)

    ok = jnp.logical_and(lmin_ref[...] >= L_LO, lmax_ref[...] <= L_HI)
    n_bad = jnp.sum(jnp.where(ok, 0.0, 1.0))

    @pl.when(n_bad > 0.0)
    def _true_max_fallback():
        def tile(g, c):
            qh = _unpack(qaug_ref[g])[0:DH]

            def scores(j):
                kb = _unpack(kaug_ref[pl.ds(pl.multiple_of(j * (BK // 2), BK // 2), BK // 2), :])
                return jnp.dot(kb[:, 0:DH], qh, preferred_element_type=f32)

            m = lax.fori_loop(
                0, NKB, lambda j, m: jnp.maximum(m, jnp.max(scores(j), axis=0, keepdims=True)),
                jnp.full((1, BQ), -jnp.inf, f32))

            def pv(j, c2):
                p = jnp.exp2(scores(j) - m)
                vb = _unpack(vt_ref[:, pl.ds(pl.multiple_of(j * BK, BK), BK)])
                return (c2[0] + jnp.dot(vb, p.astype(bf16), preferred_element_type=f32),
                        c2[1] + jnp.sum(p, axis=0, keepdims=True))

            acc, l = lax.fori_loop(0, NKB, pv,
                                   (jnp.zeros((DH, BQ), f32), jnp.zeros((1, BQ), f32)))
            ot_ref[pl.ds(pl.multiple_of((g + 1) * DH, DH), DH), :] = acc / l
            return c

        lax.fori_loop(0, NG, tile, 0)

    for c in co:
        c.wait()

    def out_copy(b, n):
        r = pl.ds(pl.multiple_of(b * BQ + n * OR, OR), OR)
        return pltpu.make_async_copy(out_ref.at[r], out_hbm.at[r], osem.at[b * OSPLIT + n])

    def out_block(b, c0):
        for n in range(OSPLIT):
            rows = pl.ds(pl.multiple_of(b * BQ + n * OR, OR), OR)
            hre = jnp.concatenate([hre_ref[c, rows, :].astype(bf16) for c in range(LT)], axis=1)
            him = jnp.concatenate([him_ref[c, rows, :].astype(bf16) for c in range(LT)], axis=1)
            y = (lax.dot_general(hre, cre_ref[...], _NT, preferred_element_type=f32)
                 - lax.dot_general(him, cim_ref[...], _NT, preferred_element_type=f32))
            o = ot_ref[pl.ds(pl.multiple_of(b * D + DH, DH), D), n * OR:(n + 1) * OR].T.astype(bf16)
            a = jnp.dot(o, wo_ref[...], preferred_element_type=f32)
            xf = x_ref[rows, :].astype(f32)
            ssm = y + xf * dskip_ref[...].astype(f32).reshape(1, D)
            g = jax.nn.sigmoid(
                jnp.sum(xf * gw_ref[...].astype(f32).reshape(1, D), axis=1, keepdims=True))
            out_ref[rows, :] = g * a + (1.0 - g) * ssm
            out_copy(b, n).start()
        return c0

    lax.fori_loop(0, NB, out_block, 0)
    for b in range(NB):
        for n in range(OSPLIT):
            out_copy(b, n).wait()


@jax.jit
def pallas_gated_mix__grouped_kv_mqa__ssm_conv_s5__prompt_kernel(
    A_x: jax.Array,
    A_wq: jax.Array,
    A_wk: jax.Array,
    A_wv: jax.Array,
    A_wo: jax.Array,
    B_x: jax.Array,
    B_Lambda_re: jax.Array,
    B_Lambda_im: jax.Array,
    B_B_re: jax.Array,
    B_B_im: jax.Array,
    B_C_re: jax.Array,
    B_C_im: jax.Array,
    B_log_dt: jax.Array,
    B_Dskip: jax.Array,
    gate_w: jax.Array,
):
    del B_x
    hbm_args = (A_x.reshape(S, D), A_wq, A_wo, B_B_re, B_B_im, B_C_re, B_C_im)
    vmem_args = (A_wk.T, A_wv.T, B_Lambda_re, B_Lambda_im, B_log_dt, B_Dskip, gate_w)

    out = pl.pallas_call(
        _kernel,
        in_specs=([pl.BlockSpec(memory_space=pl.ANY)] * len(hbm_args)
                  + [pl.BlockSpec(memory_space=pltpu.VMEM)] * len(vmem_args)),
        out_specs=pl.BlockSpec(memory_space=pl.ANY),
        out_shape=jax.ShapeDtypeStruct((S, D), f32),
        scratch_shapes=[
            pltpu.VMEM((S, D), bf16),
            pltpu.VMEM((D, D), bf16),
            pltpu.VMEM((D, D), bf16),
            pltpu.VMEM((P, D), bf16),
            pltpu.VMEM((P, D), bf16),
            pltpu.VMEM((D, P), bf16),
            pltpu.VMEM((D, P), bf16),
            pltpu.SemaphoreType.DMA((NB + 6,)),
            pltpu.SemaphoreType.DMA((NB * OSPLIT,)),
            pltpu.VMEM((S, D), f32),
            pltpu.VMEM((S // 2, 128), i32),
            pltpu.VMEM((DH // 2, S), i32),
            pltpu.VMEM((18, 8, P), f32),
            pltpu.VMEM((NG, KD // 2, BQ), i32),
            pltpu.VMEM((NG, DH, BQ), f32),
            pltpu.VMEM((DH, NVK, 128), f32),
            pltpu.VMEM((H, D), bf16),
            pltpu.VMEM((H, BQ), i32),
            pltpu.VMEM((MK // 2 + 8, BQ), i32),
            pltpu.VMEM((MK // 2 + 8, BQ), i32),
            pltpu.VMEM((NVK // 2 + 8, BQ), i32),
            pltpu.VMEM((NVK // 2 + 8, BQ), i32),
            pltpu.VMEM(((NG + 1) * DH, BQ), f32),
            pltpu.VMEM((8, BQ), f32),
            pltpu.VMEM((8, BQ), f32),
            pltpu.VMEM((LT, BQ, 128), f32),
            pltpu.VMEM((LT, BQ, 128), f32),
            pltpu.VMEM((LT, BQ, 128), f32),
            pltpu.VMEM((LT, BQ, 128), f32),
            pltpu.VMEM((LT, S, 128), f32),
            pltpu.VMEM((LT, S, 128), f32),
        ],
        compiler_params=pltpu.CompilerParams(vmem_limit_bytes=100 * 1024 * 1024),
        name="gated_mix",
    )(*hbm_args, *vmem_args)
    return out.reshape(1, S, D)
```
